```python
import os as _os
_os.environ.setdefault("JAX_PLATFORMS", "cpu")
import jax
import jax.numpy as jnp

def _softmax(x, axis=-1):
    return jax.nn.softmax(x, axis=axis)
def _gelu(x):
    return jax.nn.gelu(x, approximate=True)
def _silu(x):
    return jax.nn.silu(x)
def _sigmoid(x):
    return jax.nn.sigmoid(x)
def _layernorm(x, axis=-1, eps=1e-5):
    m = jnp.mean(x, axis=axis, keepdims=True)
    v = jnp.var(x, axis=axis, keepdims=True)
    return (x - m) / jnp.sqrt(v + eps)
def _scatter_add(tgt, idx, src, axis=0):
    return tgt.at[idx].add(src)
def _segment_sum(src, seg, n):
    return jax.ops.segment_sum(src, seg, n)
class _Rng:
    def __init__(self, key):
        self._k = key
    def _next(self):
        self._k, sub = jax.random.split(self._k)
        return sub
    def normal(self, shape):
        return jax.random.normal(self._next(), shape, dtype=jnp.bfloat16)
    def randint(self, lo, hi, shape):
        return jax.random.randint(self._next(), shape, lo, hi, dtype=jnp.int32)
    def uniform(self, shape, lo=0.0, hi=1.0):
        return jax.random.uniform(self._next(), shape, jnp.bfloat16, lo, hi)
    def permutation(self, n):
        return jax.random.permutation(self._next(), n)


kernel_name = 'interleave_layers__linear_kernel_hedgehog__dense_activation_silu__prompt'

def setup_inputs():
    _rng = _Rng(jax.random.key(int.from_bytes(__import__("os").urandom(4), "little")))
    _w = (lambda a: (lambda t: t.astype(jnp.bfloat16) if jnp.issubdtype(t.dtype, jnp.floating) else t)(jnp.asarray(a)))
    def _A_setup():
        B, S, D, H = 1, 2048, 640, 32
        Dh = D // H
        return {
            "x": _w((lambda *s: _rng.normal(s) * 0.05)(B, S, D)),
            "wqkv": _w((lambda *s: _rng.normal(s) * 0.4)(D, 3 * D)),
            "w_phi": _w((lambda *s: _rng.normal(s) * 0.4)(H, Dh, Dh) * (Dh ** -0.5)),
            "wo": _w((lambda *s: _rng.normal(s) * 0.05)(D, D)),
        }
    _A_in = _A_setup()

    def _B_setup():
        B, S, D, F = 1, 2048, 640, 1728
        return {
            "x": _w((lambda *s: _rng.normal(s) * 0.05)(B, S, D)),
            "w1": _w((lambda *s: _rng.normal(s) * 1.6)(D, F) * (D ** -0.5)),
            "w2": _w((lambda *s: _rng.normal(s) * 1.6)(F, D) * (F ** -0.5)),
        }
    _B_in = _B_setup()

    return {
        "A_x": _A_in["x"],
        "A_wqkv": _A_in["wqkv"],
        "A_w_phi": _A_in["w_phi"],
        "A_wo": _A_in["wo"],
        "B_x": _B_in["x"],
        "B_w1": _B_in["w1"],
        "B_w2": _B_in["w2"],
    }

def reference(A_x, A_wqkv, A_w_phi, A_wo, B_x, B_w1, B_w2):
    def _A_ref(x, wqkv, w_phi, wo):
        B, S, D = x.shape
        H = 32; Dh = D // H
        qkv = (lambda x, *d: x.transpose(*d))((x @ wqkv).reshape(B, S, 3, H, Dh), 2, 0, 3, 1, 4)
        q, k, v = qkv[0], qkv[1], qkv[2]
        pq = jnp.einsum("bhsd,hdf->bhsf", q, w_phi)
        pk = jnp.einsum("bhsd,hdf->bhsf", k, w_phi)
        phi_q = jnp.concatenate([_softmax(pq, axis=-1), _softmax(-pq, axis=-1)], axis=-1)
        phi_k = jnp.concatenate([_softmax(pk, axis=-1), _softmax(-pk, axis=-1)], axis=-1)
        kv = jnp.einsum("bhsf,bhsd->bhfd", phi_k, v)
        z  = jnp.einsum("bhsf->bhf", phi_k)
        num = jnp.einsum("bhqf,bhfd->bhqd", phi_q, kv)
        den = jnp.einsum("bhqf,bhf->bhq", phi_q, z)[..., None] + 1e-6
        o = num / den
        return (lambda x, *d: x.transpose(*d))(o, 0, 2, 1, 3).reshape(B, S, D) @ wo

    def _B_ref(x, w1, w2):
        h = jnp.einsum("bsd,df->bsf", x, w1)
        h = _silu(h)
        out = jnp.einsum("bsf,fd->bsd", h, w2)
        return out

    x = A_x
    x = x + _A_ref(_layernorm(x, axis=-1), A_wqkv, A_w_phi, A_wo)
    x = x + _B_ref(_layernorm(x, axis=-1), B_w1, B_w2)
    x = x + _A_ref(_layernorm(x, axis=-1), A_wqkv, A_w_phi, A_wo)
    x = x + _B_ref(_layernorm(x, axis=-1), B_w1, B_w2)
    return x
```

```python
import jax
import jax.numpy as jnp
from jax import lax
import jax.experimental.pallas as pl
import jax.experimental.pallas.tpu as pltpu

S, D, H, DH, F = 2048, 640, 32, 20, 1728
G = 4
GR = 160
SC = 512
NC = S // SC
NL = SC // 128
FB = 256
NFB = 1
RB = 64
LOG2E = 1.4426950408889634
F32, BF16 = jnp.float32, jnp.bfloat16
NT = (((1,), (1,)), ((), ()))


def _div20(i):
    return (i * 3277) >> 16


def _ln(x, scale=None):
    m = jnp.sum(x, axis=-1, keepdims=True) * (1.0 / D)
    xc = x - m
    v = jnp.sum(xc * xc, axis=-1, keepdims=True) * (1.0 / D)
    r = lax.rsqrt(v + 1e-5)
    if scale is not None:
        r = r * scale
    return (xc * r).astype(BF16)


def _dual_exp(p):
    p3 = p.reshape(DH, 8, p.shape[-1])
    mx = jnp.max(p3, axis=0, keepdims=True)
    mn = jnp.min(p3, axis=0, keepdims=True)
    ep = jnp.exp2(p3 - mx)
    en = jnp.exp2(mn - p3)
    sp = jnp.sum(ep, axis=0, keepdims=True)
    sn = jnp.sum(en, axis=0, keepdims=True)
    return ep, en, sp, sn


def _schedule():
    o = [("bd",), ("fold", 1), ("ln1", 0, 0), ("pk", 0, 0), ("wvT",), ("pv", 0, 0)]
    for c in range(NC):
        nxt = c + 1 < NC
        if nxt:
            o += [("ln1", 0, c + 1)]
        o += [("sk", 0, c, 0)]
        if nxt:
            o += [("pk", 0, c + 1)]
        o += [("sk", 0, c, 1), ("sk", 0, c, 2)]
        if nxt:
            o += [("pv", 0, c + 1)]
        o += [("sk", 0, c, 3)]
        if c == 1:
            o += [("fold", 0)]
    o += [("pq", 0, 0), ("fin", 0), ("waitw",)]
    for l in range(2):
        o += [("sq", l, 0, g) for g in range(G)]
        for c in range(NC):
            nxt = c + 1 < NC
            o += [("wo", l, c)]
            if nxt:
                o += [("pq", l, c + 1)]
            o += [("ln2", l, c)]
            side = []
            if l == 0 and c > 0:
                side += [("sk", 1, c - 1, g) for g in range(G)]
            if nxt:
                side += [("sq", l, c + 1, g) for g in range(G)]
            side = side[::-1]
            for j in range(NFB):
                o += [("fb", l, c, j)]
                if side:
                    o += [side.pop()]
            o += side[::-1]
            o += [("res", l, c)]
            if l == 0:
                o += [("ln1", 1, c), ("pkv", 1, c)]
        if l == 0:
            o += [("sk", 1, NC - 1, 0), ("pq", 1, 0)]
            o += [("sk", 1, NC - 1, g) for g in range(1, G)]
            o += [("fin", 1)]
    return o


def _kernel(x_hbm, wqkv_hbm, wphi_hbm, wo_hbm, w1_hbm, w2_hbm, out_hbm,
            xin_v, wqkv_v, wphi_v, wo_v, w1_v, w2_v, xres_v, xn_v, wt_v, obuf_v,
            kvacc_v, zacc_v, kvm_v, zb_v, wflat_v, tr_v, sems):
    def x_copy(c):
        return pltpu.make_async_copy(x_hbm.at[pl.ds(c * SC, SC)], xin_v.at[pl.ds(c * SC, SC)], sems.at[c])

    def wqkv_copy(i):
        return pltpu.make_async_copy(wqkv_hbm.at[:, pl.ds(i * D, D)], wqkv_v.at[:, pl.ds(i * D, D)], sems.at[NC + i])

    def out_copy(c):
        return pltpu.make_async_copy(obuf_v.at[pl.ds(c * SC, SC)], out_hbm.at[pl.ds(c * SC, SC)], sems.at[NC + 7 + c])
    wphi_cp = pltpu.make_async_copy(wphi_hbm, wphi_v, sems.at[NC + 3])
    wo_cp = pltpu.make_async_copy(wo_hbm, wo_v, sems.at[NC + 4])
    w1_cp = pltpu.make_async_copy(w1_hbm, w1_v, sems.at[NC + 5])
    w2_cp = pltpu.make_async_copy(w2_hbm, w2_v, sems.at[NC + 6])
    wphi_cp.start()
    wqkv_copy(1).start()
    x_copy(0).start()
    wqkv_copy(2).start()
    x_copy(1).start()
    wqkv_copy(0).start()
    for c in range(2, NC):
        x_copy(c).start()
    wo_cp.start()
    w1_cp.start()
    w2_cp.start()

    rowh = _div20(lax.broadcasted_iota(jnp.int32, (2 * DH, 4 * DH), 0))
    colh = (lax.broadcasted_iota(jnp.int32, (2 * DH, 4 * DH), 1) >> 1) & 1
    st = {}

    def to_pairs(php, phn, slot, t):
        w = pltpu.pack_elementwise([php, phn], packed_dtype=BF16)
        tr_v[slot, t] = w.reshape(GR, 128)
        return [pltpu.bitcast(tr_v[slot, t, pl.ds(p, 2 * DH, stride=4), :], BF16) for p in range(4)]

    def bd():
        wphi_cp.wait()
        for d in range(DH):
            a = jnp.pad(wphi_v[d].astype(F32), ((0, 128 - DH), (0, 128 - H)))
            wflat_v[pl.ds(d, H, stride=DH), :] = a.T[0:H]
        r = lax.broadcasted_iota(jnp.int32, (GR, 128), 0)
        fl = lax.broadcasted_iota(jnp.int32, (GR, 128), 1)
        et = jnp.where((r >> 3) == fl, 1.0, 0.0).astype(BF16)
        r2 = lax.broadcasted_iota(jnp.int32, (GR, 256), 0)
        c2 = lax.broadcasted_iota(jnp.int32, (GR, 256), 1)
        for g in range(G):
            k0 = (GR * g // 128) * 128
            b = lax.dot_general(et, wflat_v[pl.ds(k0, 256), :].astype(BF16), NT, preferred_element_type=F32)
            st["bd", g] = jnp.where(8 * g + 2 * (r2 & 3) + ((r2 >> 2) & 1) == _div20(c2 + k0), b, 0.0).astype(BF16)

    def fold(which):
        wqkv_copy(which).wait()
        for g in range(G):
            k0 = (GR * g // 128) * 128
            blk = lax.dot_general(st["bd", g], wqkv_v[:, which * D + k0:which * D + k0 + 256],
                                  NT, preferred_element_type=F32)
            wt_v[pl.ds(which * D + GR * g, GR), :] = (blk * LOG2E).astype(BF16)

    def wvT():
        wqkv_copy(2).wait()
        wt_v[pl.ds(2 * D, D), :] = wqkv_v[:, 2 * D:3 * D].T

    def waitw():
        wo_cp.wait()
        w1_cp.wait()
        w2_cp.wait()

    def ln1(l, c):
        sl = pl.ds(c * SC, SC)
        if l == 0:
            x_copy(c).wait()
            x = xin_v[sl, :].astype(F32)
        else:
            x = st["x", 0, c]
        for rb in range(SC // RB):
            xn_v[pl.ds(c * SC + rb * RB, RB), :] = _ln(x[rb * RB:(rb + 1) * RB])
        st["xn", l, c] = xn_v[sl, :]

    def pkv(l, c):
        pt = lax.dot_general(wt_v[pl.ds(D, 2 * D), :], st["xn", l, c], NT, preferred_element_type=F32)
        st["pk", l, c] = pt[0:D]
        st["pv", l, c] = pt[D:2 * D]

    def pk(l, c):
        st["pk", l, c] = lax.dot_general(wt_v[pl.ds(D, D), :], st["xn", l, c], NT, preferred_element_type=F32)

    def pv(l, c):
        st["pv", l, c] = lax.dot_general(wt_v[pl.ds(2 * D, D), :], st["xn", l, c], NT, preferred_element_type=F32)

    def sk(l, c, g):
        kvs = [None] * 4
        zc = None
        vt = st["pv", l, c]
        for t in range(NL):
            ts = slice(t * 128, (t + 1) * 128)
            ep, en, sp, sn = _dual_exp(st["pk", l, c][GR * g:GR * (g + 1), ts])
            php = ep * (1.0 / sp)
            phn = en * (1.0 / sn)
            zc = (php, phn) if zc is None else (zc[0] + php, zc[1] + phn)
            for p, ph in enumerate(to_pairs(php, phn, (c % 2) * G + g, t)):
                r0 = GR * g + 2 * DH * p
                kv = lax.dot_general(vt[r0:r0 + 2 * DH, ts].astype(BF16), ph, NT, preferred_element_type=F32)
                kvs[p] = kv if kvs[p] is None else kvs[p] + kv
        for i in range(2):
            if c == 0:
                zacc_v[g, i] = zc[i]
            else:
                zacc_v[g, i] += zc[i]
        for p in range(4):
            if c == 0:
                kvacc_v[4 * g + p] = kvs[p]
            else:
                kvacc_v[4 * g + p] += kvs[p]

    def fin(l):
        for g in range(G):
            for p in range(4):
                kvm_v[l, 4 * g + p] = jnp.where(rowh == colh, kvacc_v[4 * g + p], 0.0).astype(BF16)
            zb_v[l, g] = jnp.broadcast_to(jnp.sum(zacc_v[g], axis=-1, keepdims=True), (2, DH, 8, 128))

    def pq(l, c):
        st["pq", l, c] = lax.dot_general(wt_v[pl.ds(0, D), :], xn_v[pl.ds(c * SC, SC), :], NT,
                                         preferred_element_type=F32)

    def sq(l, c, g):
        cols = []
        for t in range(NL):
            ts = slice(t * 128, (t + 1) * 128)
            ep, en, sp, sn = _dual_exp(st["pq", l, c][GR * g:GR * (g + 1), ts])
            zp = zb_v[l, g, 0]
            zn = zb_v[l, g, 1]
            rp = 1.0 / sp
            rn = 1.0 / sn
            den = jnp.sum(ep * zp, axis=0, keepdims=True) * rp + jnp.sum(en * zn, axis=0, keepdims=True) * rn + 1e-6
            rd = 1.0 / den
            ots = [jnp.dot(kvm_v[l, 4 * g + p], ph, preferred_element_type=F32)
                   for p, ph in enumerate(to_pairs(ep * (rp * rd), en * (rn * rd), (2 + c % 2) * G + g, t))]
            cols.append(jnp.concatenate(ots, axis=0))
        st["ot", l, c, g] = jnp.concatenate(cols, axis=1)

    def wo(l, c):
        sl = pl.ds(c * SC, SC)
        o = jnp.concatenate([st["ot", l, c, g] for g in range(G)], axis=0).T.astype(BF16)
        x = xin_v[sl, :].astype(F32) if l == 0 else xres_v[sl, :]
        st["xa", l, c] = x + jnp.dot(o, wo_v[...], preferred_element_type=F32)

    def ln2(l, c):
        xa = st["xa", l, c]
        st["xn2", l, c] = jnp.concatenate([_ln(xa[rb * RB:(rb + 1) * RB], 0.5) for rb in range(SC // RB)], axis=0)

    def fb(l, c, j):
        h = lax.dot_general(st["xn2", l, c], w1_v[...], NT, preferred_element_type=F32)
        h = (h + h * jnp.tanh(h)).astype(BF16)
        st["acc", l, c] = jnp.dot(h, w2_v[...], preferred_element_type=F32)

    def res(l, c):
        sl = pl.ds(c * SC, SC)
        x = st["xa", l, c] + st["acc", l, c]
        st["x", l, c] = x
        if l == 0:
            xres_v[sl, :] = x
        else:
            obuf_v[sl, :] = x.astype(BF16)
            out_copy(c).start()

    fns = dict(bd=bd, fold=fold, wvT=wvT, waitw=waitw, ln1=ln1, pkv=pkv, pk=pk, pv=pv, sk=sk, fin=fin,
               pq=pq, sq=sq, wo=wo, ln2=ln2, fb=fb, res=res)
    for op in _schedule():
        fns[op[0]](*op[1:])
    for c in range(NC):
        out_copy(c).wait()


@jax.jit
def pallas_interleave_layers__linear_kernel_hedgehog__dense_activation_silu__prompt_kernel(
    A_x, A_wqkv, A_w_phi, A_wo, B_x, B_w1, B_w2,
):
    hbm = pl.BlockSpec(memory_space=pltpu.HBM)
    out = pl.pallas_call(
        _kernel,
        out_shape=jax.ShapeDtypeStruct((S, D), BF16),
        in_specs=[hbm] * 6,
        out_specs=hbm,
        scratch_shapes=[
            pltpu.VMEM((S, D), BF16),
            pltpu.VMEM((D, 3 * D), BF16),
            pltpu.VMEM((DH, DH, H), BF16),
            pltpu.VMEM((D, D), BF16),
            pltpu.VMEM((F, D), BF16),
            pltpu.VMEM((F, D), BF16),
            pltpu.VMEM((S, D), F32),
            pltpu.VMEM((S, D), BF16),
            pltpu.VMEM((3 * D, D), BF16),
            pltpu.VMEM((S, D), BF16),
            pltpu.VMEM((4 * G, 2 * DH, 4 * DH), F32),
            pltpu.VMEM((G, 2, DH, 8, 128), F32),
            pltpu.VMEM((2, 4 * G, 2 * DH, 4 * DH), BF16),
            pltpu.VMEM((2, G, 2, DH, 8, 128), F32),
            pltpu.VMEM((D, 128), F32),
            pltpu.VMEM((4 * G, NL, GR, 128), jnp.uint32),
            pltpu.SemaphoreType.DMA((2 * NC + 7,)),
        ],
        compiler_params=pltpu.CompilerParams(vmem_limit_bytes=100 * 1024 * 1024),
    )(A_x.reshape(S, D), A_wqkv, A_w_phi.transpose(1, 2, 0), A_wo, B_w1.T, B_w2)
    return out.reshape(1, S, D)
```

```python
import jax
import jax.numpy as jnp
from jax import lax
import jax.experimental.pallas as pl
import jax.experimental.pallas.tpu as pltpu

S, D, H, DH, F = 2048, 640, 32, 20, 1728
G = 4
GR = 160
SC = 512
NC = S // SC
NL = SC // 128
MB = 128
LOG2E = 1.4426950408889634
F32, BF16 = jnp.float32, jnp.bfloat16
NT = (((1,), (1,)), ((), ()))


def _div20(i):
    return (i * 3277) >> 16


def _ln(x, scale=None):
    m = jnp.sum(x, axis=-1, keepdims=True) * (1.0 / D)
    xc = x - m
    v = jnp.sum(xc * xc, axis=-1, keepdims=True) * (1.0 / D)
    r = lax.rsqrt(v + 1e-5)
    if scale is not None:
        r = r * scale
    return (xc * r).astype(BF16)


def _dual_exp(p):
    p3 = p.reshape(DH, 8, p.shape[-1])
    mx = jnp.max(p3, axis=0, keepdims=True)
    mn = jnp.min(p3, axis=0, keepdims=True)
    ep = jnp.exp2(p3 - mx)
    en = jnp.exp2(mn - p3)
    sp = jnp.sum(ep, axis=0, keepdims=True)
    sn = jnp.sum(en, axis=0, keepdims=True)
    return ep, en, sp, sn


def _schedule():
    o = [("bd",), ("fold", 1), ("ln1", 0, 0), ("pk", 0, 0), ("wvT",), ("pv", 0, 0)]
    for c in range(NC):
        sk = [("sk", 0, c, g) for g in range(G)]
        if c + 1 < NC:
            pk, pv = ("pk", 0, c + 1), ("pv", 0, c + 1)
            o += [("ln1", 0, c + 1)]
            o += [sk[0], pk, sk[1], sk[2], pv, sk[3]]
        else:
            o += sk + [("pq", 0, 0)]
        if c == 1:
            o += [("fold", 0)]
    o += [("fin", 0), ("waitw",)]
    for l in range(2):
        o += [("sq", l, 0, g) for g in range(G)]
        for c in range(NC):
            o += [("wo", l, c)]
            if c + 1 < NC:
                o += [("pq", l, c + 1)]
            o += [("ln2", l, c), ("fb", l, c)]
            sk = [("sk", 1, c - 1, g) for g in range(G)] if l == 0 and c > 0 else []
            sq = [("sq", l, c + 1, g) for g in range(G)] if c + 1 < NC else []
            o += sk + sq
            o += [("res", l, c)]
            if l == 0:
                o += [("ln1", 1, c), ("pkv", 1, c)]
        if l == 0:
            sk = [("sk", 1, NC - 1, g) for g in range(G)]
            o += [sk[0], ("pq", 1, 0), sk[1], sk[2]] + [sk[3], ("fin", 1)]
    return o


def _kernel(x_hbm, wqkv_hbm, wphi_hbm, wo_hbm, w1_hbm, w2_hbm, out_hbm,
            xin_v, wqkv_v, wphi_v, wo_v, w1_v, w2_v, xres_v, xn_v, wt_v, obuf_v,
            kvacc_v, zacc_v, kvm_v, zb_v, wflat_v, tr_v, sems):
    def x_copy(c):
        return pltpu.make_async_copy(x_hbm.at[pl.ds(c * SC, SC)], xin_v.at[pl.ds(c * SC, SC)], sems.at[c])

    def wqkv_copy(i):
        return pltpu.make_async_copy(wqkv_hbm.at[:, pl.ds(i * D, D)], wqkv_v.at[:, pl.ds(i * D, D)], sems.at[NC + i])

    def out_copy(r0, n, i):
        return pltpu.make_async_copy(obuf_v.at[pl.ds(r0, n)], out_hbm.at[pl.ds(r0, n)], sems.at[NC + 7 + i])

    out_cps = [out_copy(c * SC, SC, c) for c in range(NC - 1)]
    out_cps += [out_copy((NC - 1) * SC + m * MB, MB, NC - 1 + m) for m in range(SC // MB)]
    wphi_cp = pltpu.make_async_copy(wphi_hbm, wphi_v, sems.at[NC + 3])
    wo_cp = pltpu.make_async_copy(wo_hbm, wo_v, sems.at[NC + 4])
    w1_cp = pltpu.make_async_copy(w1_hbm, w1_v, sems.at[NC + 5])
    w2_cp = pltpu.make_async_copy(w2_hbm, w2_v, sems.at[NC + 6])
    wphi_cp.start()
    wqkv_copy(1).start()
    x_copy(0).start()
    wqkv_copy(2).start()
    x_copy(1).start()
    wqkv_copy(0).start()
    for c in range(2, NC):
        x_copy(c).start()
    wo_cp.start()
    w1_cp.start()
    w2_cp.start()

    rowh = _div20(lax.broadcasted_iota(jnp.int32, (2 * DH, 4 * DH), 0))
    colh = (lax.broadcasted_iota(jnp.int32, (2 * DH, 4 * DH), 1) >> 1) & 1
    st = {}

    def to_pairs(php, phn, slot, t):
        w = pltpu.pack_elementwise([php, phn], packed_dtype=BF16)
        tr_v[slot, t, pl.ds(0, GR), :] = w.reshape(GR, 128)
        return [pltpu.bitcast(tr_v[slot, t, pl.ds(p, 2 * DH, stride=4), :], BF16) for p in range(4)]

    def bd():
        wphi_cp.wait()
        for d in range(DH):
            a = jnp.pad(wphi_v[d].astype(F32), ((0, 128 - DH), (0, 128 - H)))
            wflat_v[pl.ds(d, H, stride=DH), :] = a.T[0:H]
        r = lax.broadcasted_iota(jnp.int32, (GR, 128), 0)
        fl = lax.broadcasted_iota(jnp.int32, (GR, 128), 1)
        et = jnp.where((r >> 3) == fl, 1.0, 0.0).astype(BF16)
        r2 = lax.broadcasted_iota(jnp.int32, (GR, 256), 0)
        c2 = lax.broadcasted_iota(jnp.int32, (GR, 256), 1)
        for g in range(G):
            k0 = (GR * g // 128) * 128
            b = lax.dot_general(et, wflat_v[pl.ds(k0, 256), :].astype(BF16), NT, preferred_element_type=F32)
            st["bd", g] = jnp.where(8 * g + 2 * (r2 & 3) + ((r2 >> 2) & 1) == _div20(c2 + k0), b, 0.0).astype(BF16)

    def fold(which):
        wqkv_copy(which).wait()
        for g in range(G):
            k0 = (GR * g // 128) * 128
            blk = lax.dot_general(st["bd", g], wqkv_v[:, which * D + k0:which * D + k0 + 256],
                                  NT, preferred_element_type=F32)
            wt_v[pl.ds(which * D + GR * g, GR), :] = (blk * LOG2E).astype(BF16)

    def wvT():
        wqkv_copy(2).wait()
        wt_v[pl.ds(2 * D, D), :] = wqkv_v[:, 2 * D:3 * D].T

    def waitw():
        wo_cp.wait()
        w1_cp.wait()
        w2_cp.wait()

    def ln1(l, c):
        sl = pl.ds(c * SC, SC)
        if l == 0:
            x_copy(c).wait()
            x = xin_v[sl, :].astype(F32)
        else:
            x = st["x", 0, c]
        for rb in range(SC // MB):
            xn_v[pl.ds(c * SC + rb * MB, MB), :] = _ln(x[rb * MB:(rb + 1) * MB])
        st["xn", l, c] = xn_v[sl, :]

    def pkv(l, c):
        pt = lax.dot_general(wt_v[pl.ds(D, 2 * D), :], st["xn", l, c], NT, preferred_element_type=F32)
        st["pk", l, c] = pt[0:D]
        st["pv", l, c] = pt[D:2 * D]

    def pk(l, c):
        st["pk", l, c] = lax.dot_general(wt_v[pl.ds(D, D), :], st["xn", l, c], NT, preferred_element_type=F32)

    def pv(l, c):
        st["pv", l, c] = lax.dot_general(wt_v[pl.ds(2 * D, D), :], st["xn", l, c], NT, preferred_element_type=F32)

    def sk(l, c, g):
        kvs = [None] * 4
        zc = None
        vt = st["pv", l, c]
        for t in range(NL):
            ts = slice(t * 128, (t + 1) * 128)
            ep, en, sp, sn = _dual_exp(st["pk", l, c][GR * g:GR * (g + 1), ts])
            php = ep * (1.0 / sp)
            phn = en * (1.0 / sn)
            zc = (php, phn) if zc is None else (zc[0] + php, zc[1] + phn)
            for p, ph in enumerate(to_pairs(php, phn, (c % 2) * G + g, t)):
                r0 = GR * g + 2 * DH * p
                kv = lax.dot_general(vt[r0:r0 + 2 * DH, ts].astype(BF16), ph, NT, preferred_element_type=F32)
                kvs[p] = kv if kvs[p] is None else kvs[p] + kv
        for i in range(2):
            if c == 0:
                zacc_v[g, i] = zc[i]
            else:
                zacc_v[g, i] += zc[i]
        for p in range(4):
            if c == 0:
                kvacc_v[4 * g + p] = kvs[p]
            else:
                kvacc_v[4 * g + p] += kvs[p]

    def fin(l):
        for g in range(G):
            for p in range(4):
                kvm_v[l, 4 * g + p] = jnp.where(rowh == colh, kvacc_v[4 * g + p], 0.0).astype(BF16)
            zb_v[l, g] = jnp.broadcast_to(jnp.sum(zacc_v[g], axis=-1, keepdims=True), (2, DH, 8, 128))

    def pq(l, c):
        st["pq", l, c] = lax.dot_general(wt_v[pl.ds(0, D), :], xn_v[pl.ds(c * SC, SC), :], NT,
                                         preferred_element_type=F32)

    def sq(l, c, g):
        cols = []
        for t in range(NL):
            ts = slice(t * 128, (t + 1) * 128)
            ep, en, sp, sn = _dual_exp(st["pq", l, c][GR * g:GR * (g + 1), ts])
            zp = zb_v[l, g, 0]
            zn = zb_v[l, g, 1]
            rp = 1.0 / sp
            rn = 1.0 / sn
            den = jnp.sum(ep * zp, axis=0, keepdims=True) * rp + jnp.sum(en * zn, axis=0, keepdims=True) * rn + 1e-6
            rd = 1.0 / den
            ots = [jnp.dot(kvm_v[l, 4 * g + p], ph, preferred_element_type=F32)
                   for p, ph in enumerate(to_pairs(ep * (rp * rd), en * (rn * rd), (2 + c % 2) * G + g, t))]
            cols.append(jnp.concatenate(ots, axis=0))
        st["ot", l, c, g] = jnp.concatenate(cols, axis=1)

    def wo(l, c):
        o = jnp.concatenate([st["ot", l, c, g] for g in range(G)], axis=0).T.astype(BF16)
        xs = []
        for m in range(SC // MB):
            sl = pl.ds(c * SC + m * MB, MB)
            x = xin_v[sl, :].astype(F32) if l == 0 else xres_v[sl, :]
            xs.append(x + jnp.dot(o[m * MB:(m + 1) * MB], wo_v[...], preferred_element_type=F32))
        st["xa", l, c] = xs

    def ln2(l, c):
        st["xn2", l, c] = [_ln(xa, 0.5) for xa in st["xa", l, c]]

    def fb(l, c):
        accs = []
        for xn2 in st["xn2", l, c]:
            h = lax.dot_general(xn2, w1_v[...], NT, preferred_element_type=F32)
            h = (h + h * jnp.tanh(h)).astype(BF16)
            accs.append(jnp.dot(h, w2_v[...], preferred_element_type=F32))
        st["acc", l, c] = accs

    def res(l, c):
        xs = [xa + acc for xa, acc in zip(st["xa", l, c], st["acc", l, c])]
        for m, x in enumerate(xs):
            sl = pl.ds(c * SC + m * MB, MB)
            if l == 0:
                xres_v[sl, :] = x
            else:
                obuf_v[sl, :] = x.astype(BF16)
                if c == NC - 1:
                    out_cps[NC - 1 + m].start()
        st["x", l, c] = jnp.concatenate(xs, axis=0)
        if l == 1 and c < NC - 1:
            out_cps[c].start()

    fns = dict(bd=bd, fold=fold, wvT=wvT, waitw=waitw, ln1=ln1, pkv=pkv, pk=pk, pv=pv, sk=sk, fin=fin,
               pq=pq, sq=sq, wo=wo, ln2=ln2, fb=fb, res=res)
    for op in _schedule():
        fns[op[0]](*op[1:])
    for cp in out_cps:
        cp.wait()


@jax.jit
def pallas_interleave_layers__linear_kernel_hedgehog__dense_activation_silu__prompt_kernel(
    A_x, A_wqkv, A_w_phi, A_wo, B_x, B_w1, B_w2,
):
    hbm = pl.BlockSpec(memory_space=pltpu.HBM)
    out = pl.pallas_call(
        _kernel,
        out_shape=jax.ShapeDtypeStruct((S, D), BF16),
        in_specs=[hbm] * 6,
        out_specs=hbm,
        scratch_shapes=[
            pltpu.VMEM((S, D), BF16),
            pltpu.VMEM((D, 3 * D), BF16),
            pltpu.VMEM((DH, DH, H), BF16),
            pltpu.VMEM((D, D), BF16),
            pltpu.VMEM((F, D), BF16),
            pltpu.VMEM((F, D), BF16),
            pltpu.VMEM((S, D), F32),
            pltpu.VMEM((S, D), BF16),
            pltpu.VMEM((3 * D, D), BF16),
            pltpu.VMEM((S, D), BF16),
            pltpu.VMEM((4 * G, 2 * DH, 4 * DH), F32),
            pltpu.VMEM((G, 2, DH, 8, 128), F32),
            pltpu.VMEM((2, 4 * G, 2 * DH, 4 * DH), BF16),
            pltpu.VMEM((2, G, 2, DH, 8, 128), F32),
            pltpu.VMEM((D + 24, 128), F32),
            pltpu.VMEM((4 * G, NL, GR + 8, 128), jnp.uint32),
            pltpu.SemaphoreType.DMA((2 * NC + 6 + SC // MB,)),
        ],
        compiler_params=pltpu.CompilerParams(vmem_limit_bytes=100 * 1024 * 1024),
    )(A_x.reshape(S, D), A_wqkv, A_w_phi.transpose(1, 2, 0), A_wo, B_w1.T, B_w2)
    return out.reshape(1, S, D)
```
